```python
import os as _os
_os.environ.setdefault("JAX_PLATFORMS", "cpu")
import jax
import jax.numpy as jnp

def _softmax(x, axis=-1):
    return jax.nn.softmax(x, axis=axis)
def _gelu(x):
    return jax.nn.gelu(x, approximate=True)
def _silu(x):
    return jax.nn.silu(x)
def _sigmoid(x):
    return jax.nn.sigmoid(x)
def _layernorm(x, axis=-1, eps=1e-5):
    m = jnp.mean(x, axis=axis, keepdims=True)
    v = jnp.var(x, axis=axis, keepdims=True)
    return (x - m) / jnp.sqrt(v + eps)
def _scatter_add(tgt, idx, src, axis=0):
    return tgt.at[idx].add(src)
def _segment_sum(src, seg, n):
    return jax.ops.segment_sum(src, seg, n)
class _Rng:
    def __init__(self, key):
        self._k = key
    def _next(self):
        self._k, sub = jax.random.split(self._k)
        return sub
    def normal(self, shape):
        return jax.random.normal(self._next(), shape, dtype=jnp.bfloat16)
    def randint(self, lo, hi, shape):
        return jax.random.randint(self._next(), shape, lo, hi, dtype=jnp.int32)
    def uniform(self, shape, lo=0.0, hi=1.0):
        return jax.random.uniform(self._next(), shape, jnp.bfloat16, lo, hi)
    def permutation(self, n):
        return jax.random.permutation(self._next(), n)


kernel_name = 'standalone__gqa_softmax__near_ridge'

def setup_inputs():
    _rng = _Rng(jax.random.key(int.from_bytes(__import__("os").urandom(4), "little")))
    _w = (lambda a: (lambda t: t.astype(jnp.bfloat16) if jnp.issubdtype(t.dtype, jnp.floating) else t)(jnp.asarray(a)))
    B, Hq, Hkv, Sq, Sk, D = 8, 16, 8, 512, 512, 256
    return {
        "q": _w((lambda *s: _rng.normal(s) * 0.4)(B, Hq, Sq, D)),
        "k": _w((lambda *s: _rng.normal(s) * 0.4)(B, Hkv, Sk, D)),
        "v": _w((lambda *s: _rng.normal(s) * 0.05)(B, Hkv, Sk, D)),
    }

def reference(q, k, v):
    B, Hq, Sq, D = q.shape
    Hkv = k.shape[1]
    rep = Hq // Hkv
    k = jnp.repeat(k, rep, axis=1)
    v = jnp.repeat(v, rep, axis=1)
    scale = D ** -0.5
    scores = jnp.einsum("bhqd,bhkd->bhqk", q, k) * scale
    p = _softmax(scores, axis=-1)
    return jnp.einsum("bhqk,bhkd->bhqd", p, v)
```

```python
import jax
import jax.numpy as jnp
from jax import lax
import jax.experimental.pallas as pl
import jax.experimental.pallas.tpu as pltpu

_LOG2E = 1.4426950408889634
_UNROLL = 16
_NBUF = 4


@jax.jit
def pallas_standalone__gqa_softmax__near_ridge_kernel(
    q: jax.Array,
    k: jax.Array,
    v: jax.Array,
):
    B, Hq, Sq, D = q.shape
    _, Hkv, Sk, _ = k.shape
    M = (Hq // Hkv) * Sq
    N = B * Hkv
    G, NB = _UNROLL, _NBUF
    assert G % NB == 0 and N % G == 0
    c = (D ** -0.5) * _LOG2E

    def kern(q_hbm, k_hbm, v_hbm, o_hbm, *scr):
        qb, kb, vb, ob = (scr[i * NB:(i + 1) * NB] for i in range(4))
        sem = scr[4 * NB]

        def cin(h, s):
            return (pltpu.make_async_copy(k_hbm.at[h], kb[s], sem.at[0, s]),
                    pltpu.make_async_copy(q_hbm.at[h], qb[s], sem.at[1, s]),
                    pltpu.make_async_copy(v_hbm.at[h], vb[s], sem.at[2, s]))

        def cout(h, s):
            return pltpu.make_async_copy(ob[s], o_hbm.at[h], sem.at[3, s])

        for s in range(NB):
            for cp in cin(s, s):
                cp.start()
        for cp in cin(0, 0):
            cp.wait()

        def body(it, carry):
            for g in range(G):
                h = it * G + g
                s = g % NB
                sc = lax.dot_general(qb[s][...], kb[s][...], (((1,), (1,)), ((), ())),
                                     preferred_element_type=jnp.float32)
                m = jnp.max(sc, axis=-1, keepdims=True)
                p = jnp.exp2((sc - m) * c)
                l = jnp.sum(p, axis=-1, keepdims=True)
                r = pl.reciprocal(l, approx=True)
                r = r * (2.0 - l * r)
                pb = p.astype(vb[s].dtype)
                vv = vb[s][...]

                def wait_out(h=h, s=s):
                    cout(h - NB, s).wait()

                def wait_next(h=h, g=g):
                    for cp in cin(h + 1, (g + 1) % NB):
                        cp.wait()

                def start_next(h=h, s=s):
                    for cp in cin(h + NB, s):
                        cp.start()

                if g >= NB:
                    wait_out()
                else:
                    pl.when(it > 0)(wait_out)
                if g + 1 < G:
                    wait_next()
                else:
                    pl.when(it + 1 < N // G)(wait_next)
                o = jnp.dot(pb, vv, preferred_element_type=jnp.float32)
                ob[s][...] = (o * r).astype(ob[s].dtype)
                cout(h, s).start()
                if g + NB < G:
                    start_next()
                else:
                    pl.when(it + 1 < N // G)(start_next)
            return carry

        lax.fori_loop(0, N // G, body, 0)
        for s in range(NB):
            cout(N - NB + s, s).wait()

    scratch = ([pltpu.VMEM((M, D), q.dtype)] * NB + [pltpu.VMEM((Sk, D), k.dtype)] * NB
               + [pltpu.VMEM((Sk, D), v.dtype)] * NB + [pltpu.VMEM((M, D), q.dtype)] * NB
               + [pltpu.SemaphoreType.DMA((4, NB))])
    out = pl.pallas_call(
        kern,
        in_specs=[pl.BlockSpec(memory_space=pl.ANY)] * 3,
        out_specs=pl.BlockSpec(memory_space=pl.ANY),
        out_shape=jax.ShapeDtypeStruct((N, M, D), q.dtype),
        scratch_shapes=scratch,
        compiler_params=pltpu.CompilerParams(
            vmem_limit_bytes=100 * 1024 * 1024,
            disable_bounds_checks=True,
            flags={"XLA_TPU_RESCHEDULE_DMA_DONES": True},
        ),
    )(q.reshape(N, M, D), k.reshape(N, Sk, D), v.reshape(N, Sk, D))
    return out.reshape(B, Hq, Sq, D)
```

```python
import functools
import math

import jax
import jax.numpy as jnp
from jax import lax
import jax.experimental.pallas as pl
import jax.experimental.pallas.tpu as pltpu

_LOG2E = 1.4426950408889634
_UNROLL = 16
_NBUF = 4
_ROWS = 128


def _when(cond, fn):
    if cond is True:
        fn()
    else:
        pl.when(cond)(fn)


def _attention_kernel(q_hbm, k_hbm, v_hbm, o_hbm, *scratch, unroll, nbuf, rows, exp2_scale):
    q_buf, k_buf, v_buf, o_buf = (scratch[i * nbuf:(i + 1) * nbuf] for i in range(4))
    p_buf, sems = scratch[4 * nbuf:]
    n_heads, m, _ = q_hbm.shape
    n_iters = n_heads // unroll
    chunks = [pl.ds(r, rows) for r in range(0, m, rows)]

    def k_copy(h, s):
        return pltpu.make_async_copy(k_hbm.at[h], k_buf[s], sems.at[s])

    def q_copy(h, s):
        return pltpu.make_async_copy(q_hbm.at[h], q_buf[s], sems.at[nbuf + s])

    def v_copy(h, s):
        return pltpu.make_async_copy(v_hbm.at[h], v_buf[s], sems.at[2 * nbuf + s])

    def o_copies(h, g):
        s = g % nbuf
        sem = sems.at[3 * nbuf + s]
        if g % unroll != unroll - 1:
            return [pltpu.make_async_copy(o_buf[s], o_hbm.at[h], sem)]
        return [pltpu.make_async_copy(o_buf[s].at[c], o_hbm.at[h, c], sem) for c in chunks]

    def first_q_copy(j):
        sem = sems.at[nbuf if j == 0 else 4 * nbuf + j - 1]
        return pltpu.make_async_copy(q_hbm.at[0, chunks[j]], q_buf[0].at[chunks[j]], sem)

    def start_inputs(h, s):
        k_copy(h, s).start()
        q_copy(h, s).start()
        v_copy(h, s).start()

    def wait_qk(h, s):
        k_copy(h, s).wait()
        q_copy(h, s).wait()

    def wait_output(h, g):
        for copy in o_copies(h, g):
            copy.wait()

    def one_head(it, g):
        h = it * unroll + g
        s = g % nbuf
        last = g == unroll - 1
        more_iters = it + 1 < n_iters

        scores = []
        for j, c in enumerate(chunks):
            if g == 0 and j > 0:
                pl.when(it == 0)(first_q_copy(j).wait)
            scores.append(lax.dot_general(
                q_buf[s][c, :], k_buf[s][...], (((1,), (1,)), ((), ())),
                preferred_element_type=jnp.float32))
        scores = jnp.concatenate(scores, axis=0)

        v_copy(h, s).wait()
        _when(g >= nbuf or it > 0, lambda: wait_output(h - nbuf, g - nbuf))

        row_max = jnp.max(scores, axis=-1, keepdims=True)
        p = jnp.exp2((scores - row_max) * exp2_scale)
        inv_sum = pltpu.reciprocal(jnp.sum(p, axis=-1, keepdims=True), full_range=False)
        p_buf[...] = pltpu.bitcast(p.astype(v_hbm.dtype), p_buf.dtype)
        p = pltpu.bitcast(p_buf[...], v_hbm.dtype)

        step = rows if last else m
        acc = []
        for r in range(0, m, step):
            v = v_buf[s][...]
            if r == 0:
                _when(not last or more_iters, lambda: wait_qk(h + 1, (g + 1) % nbuf))
            acc.append(jnp.dot(p[r:r + step], v, preferred_element_type=jnp.float32))
        out = (jnp.concatenate(acc, axis=0) * inv_sum).astype(o_hbm.dtype)
        for r, copy in zip(range(0, m, step), o_copies(h, g)):
            o_buf[s][pl.ds(r, step), :] = out[r:r + step]
            copy.start()
        _when(g + nbuf < unroll or more_iters, lambda: start_inputs(h + nbuf, s))

    def body(it, carry):
        for g in range(unroll):
            one_head(it, g)
        return carry

    k_copy(0, 0).start()
    for j in range(len(chunks)):
        first_q_copy(j).start()
    v_copy(0, 0).start()
    for s in range(1, nbuf):
        start_inputs(s, s)
    k_copy(0, 0).wait()
    first_q_copy(0).wait()

    lax.fori_loop(0, n_iters, body, 0)

    for h in range(n_heads - nbuf, n_heads):
        wait_output(h, h)


@jax.jit
def pallas_standalone__gqa_softmax__near_ridge_kernel(
    q: jax.Array,
    k: jax.Array,
    v: jax.Array,
):
    B, Hq, Sq, D = q.shape
    _, Hkv, Sk, _ = k.shape
    n_heads = B * Hkv
    m = (Hq // Hkv) * Sq
    unroll = math.gcd(n_heads, _UNROLL)
    assert unroll % _NBUF == 0 and m % _ROWS == 0
    packing = 4 // v.dtype.itemsize

    out = pl.pallas_call(
        functools.partial(
            _attention_kernel, unroll=unroll, nbuf=_NBUF, rows=_ROWS,
            exp2_scale=(D ** -0.5) * _LOG2E),
        in_specs=[pl.BlockSpec(memory_space=pl.ANY)] * 3,
        out_specs=pl.BlockSpec(memory_space=pl.ANY),
        out_shape=jax.ShapeDtypeStruct((n_heads, m, D), q.dtype),
        scratch_shapes=(
            [pltpu.VMEM((m, D), q.dtype)] * _NBUF
            + [pltpu.VMEM((Sk, D), k.dtype)] * _NBUF
            + [pltpu.VMEM((Sk, D), v.dtype)] * _NBUF
            + [pltpu.VMEM((m, D), q.dtype)] * _NBUF
            + [pltpu.VMEM((m // packing, Sk), jnp.uint32),
               pltpu.SemaphoreType.DMA((4 * _NBUF + m // _ROWS - 1,))]),
        compiler_params=pltpu.CompilerParams(
            vmem_limit_bytes=64 * 1024 * 1024,
            disable_bounds_checks=True,
            disable_semaphore_checks=True,
            flags={"XLA_TPU_RESCHEDULE_DMA_DONES": True},
        ),
    )(q.reshape(n_heads, m, D), k.reshape(n_heads, Sk, D), v.reshape(n_heads, Sk, D))
    return out.reshape(B, Hq, Sq, D)
```
